```python
import os as _os
_os.environ.setdefault("JAX_PLATFORMS", "cpu")
import jax
import jax.numpy as jnp

def _softmax(x, axis=-1):
    return jax.nn.softmax(x, axis=axis)
def _gelu(x):
    return jax.nn.gelu(x, approximate=True)
def _silu(x):
    return jax.nn.silu(x)
def _sigmoid(x):
    return jax.nn.sigmoid(x)
def _layernorm(x, axis=-1, eps=1e-5):
    m = jnp.mean(x, axis=axis, keepdims=True)
    v = jnp.var(x, axis=axis, keepdims=True)
    return (x - m) / jnp.sqrt(v + eps)
def _scatter_add(tgt, idx, src, axis=0):
    return tgt.at[idx].add(src)
def _segment_sum(src, seg, n):
    return jax.ops.segment_sum(src, seg, n)
class _Rng:
    def __init__(self, key):
        self._k = key
    def _next(self):
        self._k, sub = jax.random.split(self._k)
        return sub
    def normal(self, shape):
        return jax.random.normal(self._next(), shape, dtype=jnp.bfloat16)
    def randint(self, lo, hi, shape):
        return jax.random.randint(self._next(), shape, lo, hi, dtype=jnp.int32)
    def uniform(self, shape, lo=0.0, hi=1.0):
        return jax.random.uniform(self._next(), shape, jnp.bfloat16, lo, hi)
    def permutation(self, n):
        return jax.random.permutation(self._next(), n)


kernel_name = 'standalone__gqa_softmax__decode'

def setup_inputs():
    _rng = _Rng(jax.random.key(int.from_bytes(__import__("os").urandom(4), "little")))
    _w = (lambda a: (lambda t: t.astype(jnp.bfloat16) if jnp.issubdtype(t.dtype, jnp.floating) else t)(jnp.asarray(a)))
    B, Hq, Hkv, Sq, Sk, D = 8, 32, 32, 1, 4096, 128
    return {
        "q": _w((lambda *s: _rng.normal(s) * 0.4)(B, Hq, Sq, D)),
        "k": _w((lambda *s: _rng.normal(s) * 0.4)(B, Hkv, Sk, D)),
        "v": _w((lambda *s: _rng.normal(s) * 0.05)(B, Hkv, Sk, D)),
    }

def reference(q, k, v):
    B, Hq, Sq, D = q.shape
    Hkv = k.shape[1]
    rep = Hq // Hkv
    k = jnp.repeat(k, rep, axis=1)
    v = jnp.repeat(v, rep, axis=1)
    scale = D ** -0.5
    scores = jnp.einsum("bhqd,bhkd->bhqk", q, k) * scale
    p = _softmax(scores, axis=-1)
    return jnp.einsum("bhqk,bhkd->bhqd", p, v)
```

```python
import jax
import jax.numpy as jnp
from jax import lax
import jax.experimental.pallas as pl
import jax.experimental.pallas.tpu as pltpu

_G = 8
_RB = 256
_SMALL = 32
_R = 2


def _kernel(q_ref, k_hbm, v_hbm, o_ref, kbuf, vbuf, sems, qf, of):
    NH, S, D = k_hbm.shape
    G, RB, R = _G, _RB, _R
    NR = S // RB
    T = (NH // G) * NR
    AH = R - 1
    scale = D ** -0.5

    qf[...] = q_ref[...].astype(jnp.float32)

    def copies(t, si):
        g, is_v = divmod(si, 2)
        src, dst = (v_hbm, vbuf) if is_v else (k_hbm, kbuf)
        h = (t // NR) * G + g
        r0 = (t % NR) * RB
        slot = t % R
        c0 = pltpu.make_async_copy(src.at[h, pl.ds(r0, _SMALL)],
                                   dst.at[slot, g, pl.ds(0, _SMALL)],
                                   sems.at[slot, 2 * si])
        c1 = pltpu.make_async_copy(src.at[h, pl.ds(r0 + _SMALL, RB - _SMALL)],
                                   dst.at[slot, g, pl.ds(_SMALL, RB - _SMALL)],
                                   sems.at[slot, 2 * si + 1])
        return c0, c1

    def start(t, si):
        c0, c1 = copies(t, si)
        c0.start(priority=0)
        c1.start(priority=1)

    for t0 in range(AH):
        for si in range(2 * G):
            start(t0, si)

    row_s = lax.broadcasted_iota(jnp.int32, (G, RB), 0)
    row_o = lax.broadcasted_iota(jnp.int32, (G, D), 0)

    def body(t, carry):
        m, l, acc = carry
        base = pl.multiple_of((t // NR) * G, G)
        r = t % NR
        slot = t % R

        for si in range(2 * G):
            c0, c1 = copies(t, si)
            c0.wait()
            c1.wait()

            @pl.when(t + AH < T)
            def _():
                start(t + AH, si)

        first = r == 0
        m = jnp.where(first, -jnp.inf, m)
        l = jnp.where(first, 0.0, l)
        acc = jnp.where(first, 0.0, acc)

        q = qf[pl.ds(base, G), :].astype(jnp.bfloat16)
        s = jnp.zeros((G, RB), jnp.float32)
        for g in range(G):
            sg = lax.dot_general(q, kbuf[slot, g], (((1,), (1,)), ((), ())),
                                 preferred_element_type=jnp.float32)
            s = jnp.where(row_s == g, sg, s)
        s = s * scale
        m_new = jnp.maximum(m, jnp.max(s, axis=-1, keepdims=True))
        alpha = jnp.exp(m - m_new)
        p = jnp.exp(s - m_new)
        l = alpha * l + jnp.sum(p, axis=-1, keepdims=True)
        pb = p.astype(jnp.bfloat16)
        pv = jnp.zeros((G, D), jnp.float32)
        for g in range(G):
            og = jnp.dot(pb, vbuf[slot, g], preferred_element_type=jnp.float32)
            pv = jnp.where(row_o == g, og, pv)
        acc = alpha * acc + pv

        @pl.when(r == NR - 1)
        def _():
            of[pl.ds(base, G), :] = acc / l

        return m_new, l, acc

    init = (jnp.full((G, 1), -jnp.inf, jnp.float32),
            jnp.zeros((G, 1), jnp.float32),
            jnp.zeros((G, D), jnp.float32))
    lax.fori_loop(0, T, body, init)
    o_ref[...] = of[...].astype(o_ref.dtype)


@jax.jit
def pallas_standalone__gqa_softmax__decode_kernel(
    q: jax.Array,
    k: jax.Array,
    v: jax.Array,
):
    B, H, Sq, D = q.shape
    S = k.shape[2]
    NH = B * H
    out = pl.pallas_call(
        _kernel,
        in_specs=[
            pl.BlockSpec(memory_space=pltpu.VMEM),
            pl.BlockSpec(memory_space=pl.ANY),
            pl.BlockSpec(memory_space=pl.ANY),
        ],
        out_specs=pl.BlockSpec(memory_space=pltpu.VMEM),
        out_shape=jax.ShapeDtypeStruct((NH, D), q.dtype),
        scratch_shapes=[
            pltpu.VMEM((_R, _G, _RB, D), k.dtype),
            pltpu.VMEM((_R, _G, _RB, D), v.dtype),
            pltpu.SemaphoreType.DMA((_R, 4 * _G)),
            pltpu.VMEM((NH, D), jnp.float32),
            pltpu.VMEM((NH, D), jnp.float32),
        ],
    )(q.reshape(NH, D), k.reshape(NH, S, D), v.reshape(NH, S, D))
    return out.reshape(B, H, Sq, D)
```

```python
import functools

import jax
import jax.numpy as jnp
from jax import lax
import jax.experimental.pallas as pl
import jax.experimental.pallas.tpu as pltpu

_G = 16
_RB = 128
_PIECES = ((32, 0), (96, 1))
_R = 3


def _kernel(q_hbm, k_hbm, v_hbm, o_ref, kbuf, vbuf, sems, qv, qsem, qf, of):
    NH, S, D = k_hbm.shape
    G, RB, R = _G, _RB, _R
    NR = S // RB
    LOG_NR = NR.bit_length() - 1
    T = (NH // G) * NR
    AH = R - 1
    NS = G // 8
    scale = D ** -0.5

    def start(t, slot):
        h0 = (t >> LOG_NR) * G
        r0 = (t & (NR - 1)) * RB
        for g in range(G):
            for is_v, (src, dst) in enumerate(((k_hbm, kbuf), (v_hbm, vbuf))):
                off = 0
                for n, prio in _PIECES:
                    pltpu.make_async_copy(
                        src.at[h0 + g, pl.ds(r0 + off, n)],
                        dst.at[slot, g, pl.ds(off, n)],
                        sems.at[slot, is_v]).start(priority=prio)
                    off += n

    def wait(slot):
        pltpu.make_async_copy(kbuf.at[slot], kbuf.at[slot], sems.at[slot, 0]).wait()
        pltpu.make_async_copy(vbuf.at[slot], vbuf.at[slot], sems.at[slot, 1]).wait()

    for t0 in range(AH):
        start(t0, t0 % R)

    q_copy = pltpu.make_async_copy(q_hbm, qv, qsem)
    q_copy.start()
    q_copy.wait()
    qf[...] = qv[...].astype(jnp.float32)

    row = lax.broadcasted_iota(jnp.int32, (8, RB), 0)

    def compute(t, slot, carry):
        grp = t >> LOG_NR
        r = t & (NR - 1)
        first = r == 0
        new = []
        for sb in range(NS):
            m, l, acc = carry[sb]
            m = jnp.where(first, -jnp.inf, m)
            l = jnp.where(first, 0.0, l)
            acc = jnp.where(first, 0.0, acc)
            base = pl.multiple_of(grp * G + sb * 8, 8)
            q = qf[pl.ds(base, 8), :].astype(jnp.bfloat16)
            kk = kbuf[slot, sb * 8:(sb + 1) * 8].reshape(8 * RB, D)
            s_all = lax.dot_general(q, kk, (((1,), (1,)), ((), ())),
                                    preferred_element_type=jnp.float32)
            s = s_all[:, 0:RB]
            for g in range(1, 8):
                s = jnp.where(row == g, s_all[:, g * RB:(g + 1) * RB], s)
            s = s * scale
            m_new = jnp.maximum(m, jnp.max(s, axis=-1, keepdims=True))
            alpha = jnp.exp(m - m_new)
            p = jnp.exp(s - m_new)
            l = alpha * l + p
            p_diag = jnp.concatenate(
                [jnp.where(row == g, p, 0.0).astype(jnp.bfloat16) for g in range(8)],
                axis=1)
            vv = vbuf[slot, sb * 8:(sb + 1) * 8].reshape(8 * RB, D)
            pv = jnp.dot(p_diag, vv, preferred_element_type=jnp.float32)
            acc = alpha * acc + pv
            new.append((m_new, l, acc))

        @pl.when(r == NR - 1)
        def _():
            for sb in range(NS):
                base = pl.multiple_of(grp * G + sb * 8, 8)
                _, l, acc = new[sb]
                of[pl.ds(base, 8), :] = acc / jnp.sum(l, axis=-1, keepdims=True)

        return tuple(new)

    def body(t, carry, prefetch=True):
        slot = lax.rem(t, R)
        wait(slot)
        if prefetch:
            start(t + AH, lax.rem(t + AH, R))
        return compute(t, slot, carry)

    init = tuple((jnp.full((8, 1), -jnp.inf, jnp.float32),
                  jnp.zeros((8, RB), jnp.float32),
                  jnp.zeros((8, D), jnp.float32)) for _ in range(NS))
    carry = lax.fori_loop(0, T - AH, body, init)
    lax.fori_loop(T - AH, T, functools.partial(body, prefetch=False), carry)
    o_ref[...] = of[...].astype(o_ref.dtype)


@jax.jit
def pallas_standalone__gqa_softmax__decode_kernel(
    q: jax.Array,
    k: jax.Array,
    v: jax.Array,
):
    B, H, Sq, D = q.shape
    S = k.shape[2]
    NH = B * H
    assert Sq == 1 and k.shape == (B, H, S, D) and v.shape == k.shape
    assert NH % _G == 0 and S % _RB == 0 and (S // _RB) & (S // _RB - 1) == 0
    out = pl.pallas_call(
        _kernel,
        in_specs=[
            pl.BlockSpec(memory_space=pl.ANY),
            pl.BlockSpec(memory_space=pl.ANY),
            pl.BlockSpec(memory_space=pl.ANY),
        ],
        out_specs=pl.BlockSpec(memory_space=pltpu.VMEM),
        out_shape=jax.ShapeDtypeStruct((NH, D), q.dtype),
        scratch_shapes=[
            pltpu.VMEM((_R, _G, _RB, D), k.dtype),
            pltpu.VMEM((_R, _G, _RB, D), v.dtype),
            pltpu.SemaphoreType.DMA((_R, 2)),
            pltpu.VMEM((NH, D), q.dtype),
            pltpu.SemaphoreType.DMA(()),
            pltpu.VMEM((NH, D), jnp.float32),
            pltpu.VMEM((NH, D), jnp.float32),
        ],
    )(q.reshape(NH, D), k.reshape(NH, S, D), v.reshape(NH, S, D))
    return out.reshape(B, H, Sq, D)
```

```python
import functools

import jax
import jax.numpy as jnp
from jax import lax
import jax.experimental.pallas as pl
import jax.experimental.pallas.tpu as pltpu

_G = 16
_RB = 128
_PIECES = ((32, 0), (96, 1))
_R = 3


def _kernel(q_hbm, k_hbm, v_hbm, o_ref, kbuf, vbuf, sems, qv, qsem, qf, of):
    NH, S, D = k_hbm.shape
    G, RB, R = _G, _RB, _R
    NR = S // RB
    LOG_NR = NR.bit_length() - 1
    T = (NH // G) * NR
    AH = R - 1
    NS = G // 8
    scale = D ** -0.5

    def start(t, slot):
        h0 = (t >> LOG_NR) * G
        r0 = (t & (NR - 1)) * RB
        for g in range(G):
            for is_v, (src, dst) in enumerate(((k_hbm, kbuf), (v_hbm, vbuf))):
                off = 0
                for n, prio in _PIECES:
                    pltpu.make_async_copy(
                        src.at[h0 + g, pl.ds(r0 + off, n)],
                        dst.at[slot, g, pl.ds(off, n)],
                        sems.at[slot, 2 * (g // 8) + is_v]).start(priority=prio)
                    off += n

    def wait(slot, sb):
        sl = pl.ds(sb * 8, 8)
        pltpu.make_async_copy(kbuf.at[slot, sl], kbuf.at[slot, sl], sems.at[slot, 2 * sb]).wait()
        pltpu.make_async_copy(vbuf.at[slot, sl], vbuf.at[slot, sl], sems.at[slot, 2 * sb + 1]).wait()

    for t0 in range(AH):
        start(t0, t0 % R)

    q_copy = pltpu.make_async_copy(q_hbm, qv, qsem)
    q_copy.start()
    q_copy.wait()
    qf[...] = qv[...].astype(jnp.float32)

    row = lax.broadcasted_iota(jnp.int32, (8, RB), 0)

    def compute(t, slot, carry, split=False):
        grp = t >> LOG_NR
        r = t & (NR - 1)
        first = r == 0
        new = []
        for sb in range(NS):
            if split:
                wait(slot, sb)
            m, l, acc = carry[sb]
            m = jnp.where(first, -jnp.inf, m)
            l = jnp.where(first, 0.0, l)
            acc = jnp.where(first, 0.0, acc)
            base = pl.multiple_of(grp * G + sb * 8, 8)
            q = qf[pl.ds(base, 8), :].astype(jnp.bfloat16)
            kk = kbuf[slot, sb * 8:(sb + 1) * 8].reshape(8 * RB, D)
            s_all = lax.dot_general(q, kk, (((1,), (1,)), ((), ())),
                                    preferred_element_type=jnp.float32)
            s = s_all[:, 0:RB]
            for g in range(1, 8):
                s = jnp.where(row == g, s_all[:, g * RB:(g + 1) * RB], s)
            s = s * scale
            m_new = jnp.maximum(m, jnp.max(s, axis=-1, keepdims=True))
            alpha = jnp.exp(m - m_new)
            p = jnp.exp(s - m_new)
            l = alpha * l + p
            p_diag = jnp.concatenate(
                [jnp.where(row == g, p, 0.0).astype(jnp.bfloat16) for g in range(8)],
                axis=1)
            vv = vbuf[slot, sb * 8:(sb + 1) * 8].reshape(8 * RB, D)
            pv = jnp.dot(p_diag, vv, preferred_element_type=jnp.float32)
            acc = alpha * acc + pv
            new.append((m_new, l, acc))

        @pl.when(r == NR - 1)
        def _():
            for sb in range(NS):
                base = pl.multiple_of(grp * G + sb * 8, 8)
                _, l, acc = new[sb]
                of[pl.ds(base, 8), :] = acc / jnp.sum(l, axis=-1, keepdims=True)

        return tuple(new)

    def body(t, carry, prefetch=True):
        slot = lax.rem(t, R)
        if prefetch:
            for sb in range(NS):
                wait(slot, sb)
            start(t + AH, lax.rem(t + AH, R))
        return compute(t, slot, carry, split=not prefetch)

    init = tuple((jnp.full((8, 1), -jnp.inf, jnp.float32),
                  jnp.zeros((8, RB), jnp.float32),
                  jnp.zeros((8, D), jnp.float32)) for _ in range(NS))
    carry = lax.fori_loop(0, T - AH, body, init)
    lax.fori_loop(T - AH, T, functools.partial(body, prefetch=False), carry)
    o_ref[...] = of[...].astype(o_ref.dtype)


@jax.jit
def pallas_standalone__gqa_softmax__decode_kernel(
    q: jax.Array,
    k: jax.Array,
    v: jax.Array,
):
    B, H, Sq, D = q.shape
    S = k.shape[2]
    NH = B * H
    assert Sq == 1 and k.shape == (B, H, S, D) and v.shape == k.shape
    assert NH % _G == 0 and S % _RB == 0 and (S // _RB) & (S // _RB - 1) == 0
    out = pl.pallas_call(
        _kernel,
        in_specs=[
            pl.BlockSpec(memory_space=pl.ANY),
            pl.BlockSpec(memory_space=pl.ANY),
            pl.BlockSpec(memory_space=pl.ANY),
        ],
        out_specs=pl.BlockSpec(memory_space=pltpu.VMEM),
        out_shape=jax.ShapeDtypeStruct((NH, D), q.dtype),
        scratch_shapes=[
            pltpu.VMEM((_R, _G, _RB, D), k.dtype),
            pltpu.VMEM((_R, _G, _RB, D), v.dtype),
            pltpu.SemaphoreType.DMA((_R, 2 * (_G // 8))),
            pltpu.VMEM((NH, D), q.dtype),
            pltpu.SemaphoreType.DMA(()),
            pltpu.VMEM((NH, D), jnp.float32),
            pltpu.VMEM((NH, D), jnp.float32),
        ],
    )(q.reshape(NH, D), k.reshape(NH, S, D), v.reshape(NH, S, D))
    return out.reshape(B, H, Sq, D)
```
